```python
import os as _os
_os.environ.setdefault("JAX_PLATFORMS", "cpu")
import jax
import jax.numpy as jnp

def _softmax(x, axis=-1):
    return jax.nn.softmax(x, axis=axis)
def _gelu(x):
    return jax.nn.gelu(x, approximate=True)
def _silu(x):
    return jax.nn.silu(x)
def _sigmoid(x):
    return jax.nn.sigmoid(x)
def _layernorm(x, axis=-1, eps=1e-5):
    m = jnp.mean(x, axis=axis, keepdims=True)
    v = jnp.var(x, axis=axis, keepdims=True)
    return (x - m) / jnp.sqrt(v + eps)
def _scatter_add(tgt, idx, src, axis=0):
    return tgt.at[idx].add(src)
def _segment_sum(src, seg, n):
    return jax.ops.segment_sum(src, seg, n)
class _Rng:
    def __init__(self, key):
        self._k = key
    def _next(self):
        self._k, sub = jax.random.split(self._k)
        return sub
    def normal(self, shape):
        return jax.random.normal(self._next(), shape, dtype=jnp.bfloat16)
    def randint(self, lo, hi, shape):
        return jax.random.randint(self._next(), shape, lo, hi, dtype=jnp.int32)
    def uniform(self, shape, lo=0.0, hi=1.0):
        return jax.random.uniform(self._next(), shape, jnp.bfloat16, lo, hi)
    def permutation(self, n):
        return jax.random.permutation(self._next(), n)


kernel_name = 'sequential_preLN__linear_attn_block__glu_gated_reglu__prompt'

def setup_inputs():
    _rng = _Rng(jax.random.key(int.from_bytes(__import__("os").urandom(4), "little")))
    _w = (lambda a: (lambda t: t.astype(jnp.bfloat16) if jnp.issubdtype(t.dtype, jnp.floating) else t)(jnp.asarray(a)))
    def _A_setup():
        B, S, D = 1, 2048, 640
        return {
            "x": _w((lambda *s: _rng.normal(s) * 0.05)(B, S, D)),
            "wqkv": _w((lambda *s: _rng.normal(s) * 0.05)(D, 3 * D)),
            "wo": _w((lambda *s: _rng.normal(s) * 0.05)(D, D)),
        }
    _A_in = _A_setup()

    def _B_setup():
        B, S, D, F = 1, 2048, 640, 1536
        return {
            "x": _w((lambda *s: _rng.normal(s) * 0.05)(B, S, D)),
            "W_gate": _w((lambda *s: _rng.normal(s) * 0.05)(D, F) * (2.0 / D) ** 0.5),
            "W_up": _w((lambda *s: _rng.normal(s) * 0.05)(D, F) * (2.0 / D) ** 0.5),
            "W_down": _w((lambda *s: _rng.normal(s) * 0.05)(F, D) * (1.0 / F) ** 0.5),
        }
    _B_in = _B_setup()

    return {
        "A_x": _A_in["x"],
        "A_wqkv": _A_in["wqkv"],
        "A_wo": _A_in["wo"],
        "B_x": _B_in["x"],
        "B_W_gate": _B_in["W_gate"],
        "B_W_up": _B_in["W_up"],
        "B_W_down": _B_in["W_down"],
    }

def reference(A_x, A_wqkv, A_wo, B_x, B_W_gate, B_W_up, B_W_down):
    def _A_ref(x, wqkv, wo):
        B, S, D = x.shape
        H = 32; Dh = D // H
        qkv = (lambda x, *d: x.transpose(*d))((x @ wqkv).reshape(B, S, 3, H, Dh), 2, 0, 3, 1, 4)
        q, k, v = qkv[0], qkv[1], qkv[2]
        phi = lambda t: jnp.where(t > 0, t + 1, jnp.exp(t)) + 1e-6
        pq, pk = phi(q), phi(k)
        kv = jnp.einsum("bhsd,bhse->bhde", pk, v)
        z = jnp.einsum("bhsd->bhd", pk)
        num = jnp.einsum("bhqd,bhde->bhqe", pq, kv)
        den = jnp.einsum("bhqd,bhd->bhq", pq, z)[..., None] + 1e-6
        o = num / den
        return (lambda x, *d: x.transpose(*d))(o, 0, 2, 1, 3).reshape(B, S, D) @ wo

    def _B_ref(x, W_gate, W_up, W_down):
        gate = jnp.einsum("bsd,df->bsf", x, W_gate)
        up = jnp.einsum("bsd,df->bsf", x, W_up)
        gate = gate * (lambda x, dt: x.astype(dt))(gate > 0, gate.dtype)
        h = gate * up
        return jnp.einsum("bsf,fd->bsd", h, W_down)

    x = A_x
    h = x + _A_ref(_layernorm(x, axis=-1), A_wqkv, A_wo)
    h2 = h + _B_ref(_layernorm(h, axis=-1), B_W_gate, B_W_up, B_W_down)
    return h2
```

```python
import functools
import jax
import jax.numpy as jnp
from jax import lax
import jax.experimental.pallas as pl
import jax.experimental.pallas.tpu as pltpu

S = 2048
D = 640
F = 1536
H = 32
DH = 20
TM = 512
NB = S // TM
NT = D // 128

def _band(j):
    h0 = (128 * j) // DH
    h1 = (128 * j + 127) // DH
    r0 = (h0 * DH) // 16 * 16
    r1 = -(-((h1 + 1) * DH) // 16) * 16
    return r0, min(r1, D)

BANDS = [_band(j) for j in range(NT)]
BW = max(r1 - r0 for r0, r1 in BANDS)


def _ln(x):
    mu = jnp.mean(x, axis=-1, keepdims=True)
    xc = x - mu
    var = jnp.mean(xc * xc, axis=-1, keepdims=True)
    return xc * lax.rsqrt(var + 1e-5)


def _phi(t):
    return jnp.where(t > 0, t + 1.0, jnp.exp(t)) + 1e-6


def _kernel(x_ref, wqkv_hbm, wo_hbm, wg_hbm, wu_hbm, wd_hbm, o_ref,
            wqkv, wo, wg, wu, wd, wkT, pq_scr, kv_acc, z_acc, m_scr, zs_scr, e_scr, sems):
    p = pl.program_id(0)
    i = pl.program_id(1)
    f32 = jnp.float32
    bf16 = jnp.bfloat16

    def copies():
        return [pltpu.make_async_copy(src, dst, sems.at[n])
                for n, (src, dst) in enumerate(
                    [(wqkv_hbm, wqkv), (wo_hbm, wo), (wg_hbm, wg), (wu_hbm, wu), (wd_hbm, wd)])]

    @pl.when(jnp.logical_and(p == 0, i == 0))
    def _():
        cs = copies()
        for c in cs:
            c.start()
        kv_acc[...] = jnp.zeros(kv_acc.shape, f32)
        z_acc[...] = jnp.zeros(z_acc.shape, f32)
        cs[0].wait()
        wkT[...] = wqkv[:, D:2 * D].astype(f32).T.astype(bf16)

    @pl.when(p == 0)
    def _():
        xn = _ln(x_ref[...].astype(f32)).astype(bf16)
        q = jnp.dot(xn, wqkv[:, 0:D], preferred_element_type=f32)
        pq_scr[pl.ds(pl.multiple_of(i * TM, TM), TM), :] = _phi(q).astype(bf16)
        v = jnp.dot(xn, wqkv[:, 2 * D:3 * D], preferred_element_type=f32).astype(bf16)
        kT = lax.dot_general(wkT[...], xn, (((1,), (1,)), ((), ())), preferred_element_type=f32)
        pkT = _phi(kT)
        zs = pkT[:, 0:128]
        for t in range(1, TM // 128):
            zs = zs + pkT[:, 128 * t:128 * (t + 1)]
        z_acc[...] += zs
        pkb = pkT.astype(bf16)
        for j, (r0, r1) in enumerate(BANDS):
            kv_acc[j, 0:r1 - r0, :] += jnp.dot(pkb[r0:r1, :], v[:, 128 * j:128 * (j + 1)],
                                               preferred_element_type=f32)

    @pl.when(jnp.logical_and(p == 1, i == 0))
    def _():
        cs = copies()
        for c in cs[1:]:
            c.wait()
        m_scr[...] = jnp.zeros(m_scr.shape, f32)
        for j, (r0, r1) in enumerate(BANDS):
            n = r1 - r0
            rh = (lax.broadcasted_iota(jnp.int32, (n, 128), 0) + r0) // DH
            ch = (lax.broadcasted_iota(jnp.int32, (n, 128), 1) + 128 * j) // DH
            kvj = jnp.where(rh == ch, kv_acc[j, 0:n, :], 0.0).astype(bf16)
            m_scr[r0:r1, :] += jnp.dot(kvj, wo[128 * j:128 * (j + 1), :], preferred_element_type=f32)
        z = jnp.sum(z_acc[...], axis=-1, keepdims=True)
        rh = lax.broadcasted_iota(jnp.int32, (D, 128), 0) // DH
        ch = lax.broadcasted_iota(jnp.int32, (D, 128), 1) % H
        zs_scr[...] = jnp.where(rh == ch, z, 0.0).astype(bf16)
        er = lax.broadcasted_iota(jnp.int32, (128, D), 0) % H
        ec = lax.broadcasted_iota(jnp.int32, (128, D), 1) // DH
        e_scr[...] = jnp.where(er == ec, 1.0, 0.0).astype(bf16)

    @pl.when(p == 1)
    def _():
        pq = pq_scr[pl.ds(pl.multiple_of(i * TM, TM), TM), :]
        den = jnp.dot(pq, zs_scr[...], preferred_element_type=f32) + 1e-6
        r = 1.0 / den
        hi = r.astype(bf16).astype(f32)
        lo = (r - hi).astype(bf16).astype(f32)
        lo2 = r - hi - lo
        lane = lax.broadcasted_iota(jnp.int32, (TM, 128), 1)
        sel = jnp.where(lane < H, hi, jnp.where(lane < 2 * H, lo, jnp.where(lane < 3 * H, lo2, 0.0)))
        rexp = jnp.dot(sel.astype(bf16), e_scr[...], preferred_element_type=f32)
        pqn = (pq.astype(f32) * rexp).astype(bf16)
        attn = jnp.dot(pqn, m_scr[...].astype(bf16), preferred_element_type=f32)
        h = x_ref[...].astype(f32) + attn
        hn = _ln(h).astype(bf16)
        g = jnp.dot(hn, wg[...], preferred_element_type=f32)
        u = jnp.dot(hn, wu[...], preferred_element_type=f32)
        a = (jnp.maximum(g, 0.0) * u).astype(bf16)
        o_ref[...] = (h + jnp.dot(a, wd[...], preferred_element_type=f32)).astype(o_ref.dtype)


@jax.jit
def pallas_sequential_preLN__linear_attn_block__glu_gated_reglu__prompt_kernel(
    A_x, A_wqkv, A_wo, B_x, B_W_gate, B_W_up, B_W_down,
):
    bf16 = jnp.bfloat16
    f32 = jnp.float32
    x = A_x.reshape(S, D)
    any_spec = pl.BlockSpec(memory_space=pl.ANY)
    out = pl.pallas_call(
        _kernel,
        grid=(2, NB),
        in_specs=[pl.BlockSpec((TM, D), lambda p, i: (i, 0)),
                  any_spec, any_spec, any_spec, any_spec, any_spec],
        out_specs=pl.BlockSpec((TM, D), lambda p, i: (i * p, 0)),
        out_shape=jax.ShapeDtypeStruct((S, D), A_x.dtype),
        scratch_shapes=[
            pltpu.VMEM((D, 3 * D), bf16),
            pltpu.VMEM((D, D), bf16),
            pltpu.VMEM((D, F), bf16),
            pltpu.VMEM((D, F), bf16),
            pltpu.VMEM((F, D), bf16),
            pltpu.VMEM((D, D), bf16),
            pltpu.VMEM((S, D), bf16),
            pltpu.VMEM((NT, BW, 128), f32),
            pltpu.VMEM((D, 128), f32),
            pltpu.VMEM((D, D), f32),
            pltpu.VMEM((D, 128), bf16),
            pltpu.VMEM((128, D), bf16),
            pltpu.SemaphoreType.DMA((5,)),
        ],
        compiler_params=pltpu.CompilerParams(
            dimension_semantics=("arbitrary", "arbitrary"),
            vmem_limit_bytes=100 * 1024 * 1024,
        ),
    )(x, A_wqkv, A_wo, B_W_gate, B_W_up, B_W_down)
    return out.reshape(A_x.shape)
```

```python
import functools
import jax
import jax.numpy as jnp
from jax import lax
import jax.experimental.pallas as pl
import jax.experimental.pallas.tpu as pltpu

S = 2048
D = 640
F = 1536
H = 32
DH = 20
TM = 512
NB = S // TM
NT = D // 128
NP = H // 2
NC = TM // 128
FC = F // NC

def _band(j):
    h0 = (128 * j) // DH
    h1 = (128 * j + 127) // DH
    r0 = (h0 * DH) // 16 * 16
    r1 = -(-((h1 + 1) * DH) // 16) * 16
    return r0, min(r1, D)

BANDS = [_band(j) for j in range(NT)]


def _ln(x):
    mu = jnp.mean(x, axis=-1, keepdims=True)
    xc = x - mu
    var = jnp.mean(xc * xc, axis=-1, keepdims=True)
    return xc * lax.rsqrt(var + 1e-5)


def _recip(d):
    r = pl.reciprocal(d, approx=True)
    return r * (2.0 - d * r)


def _phi(t):
    return jnp.where(t > 0, t + 1.0, jnp.exp(t)) + 1e-6


def _kernel(x_hbm, wqkv_hbm, wo_hbm, wg_hbm, wu_hbm, wd_hbm, o_hbm,
            x_scr, wq, wk, wv, wo, wg, wu, wd, wkT, wqT, xn_scr, pqT_scr, g_acc, z_acc, m_scr, m_bf,
            zb_scr, h_cur, h_nxt, hn_scr, a_scr, pqn_scr, o_scr, pk_scr, sems, osems):
    s = pl.program_id(0)
    f32 = jnp.float32
    bf16 = jnp.bfloat16

    HM = TM // 2
    KS = 256
    pairs = [(x_hbm.at[pl.ds(0, HM), :], x_scr.at[0, pl.ds(0, HM), :]),
             (wqkv_hbm.at[:, D:D + KS], wk.at[:, 0:KS]),
             (wqkv_hbm.at[:, D + KS:2 * D], wk.at[:, KS:D]),
             (x_hbm.at[pl.ds(HM, HM), :], x_scr.at[0, pl.ds(HM, HM), :])]
    pairs.append((wqkv_hbm.at[:, 0:D], wq))
    IQ = len(pairs) - 1
    for b in range(1, NB):
        pairs.append((x_hbm.at[pl.ds(b * TM, TM), :], x_scr.at[b]))
    IREST = len(pairs)
    pairs += [(wqkv_hbm.at[:, 2 * D:3 * D], wv), (wo_hbm, wo), (wg_hbm, wg), (wu_hbm, wu), (wd_hbm, wd)]
    NDMA = len(pairs)

    def copy(n):
        return pltpu.make_async_copy(pairs[n][0], pairs[n][1], sems.at[n])

    def ocopy(blk, j):
        return pltpu.make_async_copy(
            o_scr.at[:, 128 * j:128 * (j + 1)],
            o_hbm.at[pl.ds(pl.multiple_of(blk * TM, TM), TM), 128 * j:128 * (j + 1)],
            osems.at[j])

    NTDIMS = (((1,), (1,)), ((), ()))

    def qproj(blk, r0=0, r1=D):
        qT = lax.dot_general(wqT[r0:r1, :], xn_scr[blk], NTDIMS, preferred_element_type=f32)
        pqT_scr[blk, r0:r1, :] = _phi(qT)

    def zsum(pkT):
        zs = pkT[:, 0:128]
        for t in range(1, NC):
            zs = zs + pkT[:, 128 * t:128 * (t + 1)]
        return zs

    def norm_piece(blk, c):
        lo = lax.broadcasted_iota(jnp.int32, (NP, 8, 128), 1) < 4
        zb5 = zb_scr[...].reshape(NP, 5, 8, 128)
        p5 = pqT_scr[blk, :, 128 * c:128 * (c + 1)].reshape(NP, 5, 8, 128)
        t5 = p5 * zb5
        ta = t5[:, 0] + t5[:, 1] + jnp.where(lo, t5[:, 2], 0.0)
        tb = jnp.where(lo, 0.0, t5[:, 2]) + t5[:, 3] + t5[:, 4]
        ra = _recip(jnp.sum(ta, axis=1, keepdims=True) + 1e-6)
        rb = _recip(jnp.sum(tb, axis=1, keepdims=True) + 1e-6)
        ra = jnp.broadcast_to(ra, (NP, 8, 128))
        rb = jnp.broadcast_to(rb, (NP, 8, 128))
        rm = jnp.where(lo, ra, rb)
        pn = jnp.stack([p5[:, 0] * ra, p5[:, 1] * ra, p5[:, 2] * rm, p5[:, 3] * rb, p5[:, 4] * rb],
                       axis=1).reshape(D, 128)
        pqn_scr[128 * c:128 * (c + 1), :] = pn.T

    def h_ln(blk, attn, r0, r1):
        h = x_scr[blk, r0:r1, :].astype(f32) + attn[r0:r1, :]
        h_nxt[r0:r1, :] = h
        hn_scr[r0:r1, :] = _ln(h).astype(bf16)

    def down_tile(blk, j):
        d = jnp.dot(a_scr[...], wd[:, 128 * j:128 * (j + 1)], preferred_element_type=f32)
        o_scr[:, 128 * j:128 * (j + 1)] = (h_cur[:, 128 * j:128 * (j + 1)] + d).astype(bf16)
        ocopy(blk, j).start()

    @pl.when(s == 0)
    @jax.named_scope("p1_first")
    def _():
        for n in range(NDMA):
            copy(n).start()

        def kpiece(r0, r1, c0, c1):
            kT = lax.dot_general(wkT[r0:r1, :], xn_scr[0, c0:c1, :], NTDIMS,
                                 preferred_element_type=f32)
            pkT = _phi(kT)
            zs = pkT[:, 0:128]
            for t in range(1, (c1 - c0) // 128):
                zs = zs + pkT[:, 128 * t:128 * (t + 1)]
            if c0 == 0:
                z_acc[r0:r1, :] = zs
            else:
                z_acc[r0:r1, :] += zs
            pk_scr[r0:r1, c0:c1] = pkT.astype(bf16)

        copy(0).wait()
        xn_scr[0, 0:HM, :] = _ln(x_scr[0, 0:HM, :].astype(f32)).astype(bf16)
        copy(1).wait()
        wkT[0:KS, :] = wk[:, 0:KS].T
        kpiece(0, KS, 0, HM)
        copy(2).wait()
        copy(3).wait()
        wkT[KS:D, :] = wk[:, KS:D].T
        xn_scr[0, HM:TM, :] = _ln(x_scr[0, HM:TM, :].astype(f32)).astype(bf16)
        kpiece(KS, D, 0, HM)
        kpiece(0, D, HM, TM)
        copy(IQ).wait()
        wqT[...] = wq[...].T
        g_acc[...] = jnp.dot(pk_scr[...], xn_scr[0], preferred_element_type=f32)

    @pl.when(jnp.logical_and(s > 0, s < NB))
    @jax.named_scope("p1_rest")
    def _():
        pltpu.make_async_copy(x_hbm.at[pl.ds(0, TM), :], x_scr.at[s], sems.at[s + IQ]).wait()
        qproj(s - 1)
        xn = _ln(x_scr[s].astype(f32)).astype(bf16)
        xn_scr[s] = xn
        kT = lax.dot_general(wkT[...], xn, NTDIMS, preferred_element_type=f32)
        pkT = _phi(kT)
        z_acc[...] += zsum(pkT)
        g_acc[...] += jnp.dot(pkT.astype(bf16), xn, preferred_element_type=f32)

    @pl.when(s == NB)
    @jax.named_scope("mid")
    def _():
        for n in range(IREST, NDMA):
            copy(n).wait()
        zb_scr[...] = jnp.broadcast_to(jnp.sum(z_acc[...], axis=1, keepdims=True), (D, 128))
        kvs = []
        for j, (r0, r1) in enumerate(BANDS):
            n = r1 - r0
            kvj = jnp.dot(g_acc[r0:r1, :].astype(bf16), wv[:, 128 * j:128 * (j + 1)],
                          preferred_element_type=f32)
            rh = (lax.broadcasted_iota(jnp.int32, (n, 128), 0) + r0) // DH
            ch = (lax.broadcasted_iota(jnp.int32, (n, 128), 1) + 128 * j) // DH
            kvs.append(jnp.where(rh == ch, kvj, 0.0).astype(bf16))
        norm_piece(0, 0)
        qproj(NB - 1, 0, 256)
        norm_piece(0, 1)
        m_scr[...] = jnp.zeros(m_scr.shape, f32)
        for j, (r0, r1) in enumerate(BANDS):
            m_scr[r0:r1, :] += jnp.dot(kvs[j], wo[128 * j:128 * (j + 1), :], preferred_element_type=f32)
        norm_piece(0, 2)
        qproj(NB - 1, 256, 384)
        norm_piece(0, 3)
        m_bf[...] = m_scr[...].astype(bf16)
        attn = jnp.dot(pqn_scr[...].astype(bf16), m_bf[...], preferred_element_type=f32)
        qproj(NB - 1, 384, 640)
        h_ln(0, attn, 0, TM)

    i = s - (NB + 1)

    @pl.when(i >= 0)
    @jax.named_scope("p2_a")
    def _():
        h_cur[...] = h_nxt[...]
        hn = hn_scr[...]
        nxt = jnp.minimum(i + 1, NB - 1)
        for c in range(NC):
            g = jnp.dot(hn, wg[:, FC * c:FC * (c + 1)], preferred_element_type=f32)
            if c > 0:
                norm_piece(nxt, c - 1)
            u = jnp.dot(hn, wu[:, FC * c:FC * (c + 1)], preferred_element_type=f32)
            if c == NC - 1:
                norm_piece(nxt, c)
            a_scr[:, FC * c:FC * (c + 1)] = (jnp.maximum(g, 0.0) * u).astype(bf16)

    @pl.when(i >= 1)
    def _():
        for j in range(NT):
            ocopy(i - 1, j).wait()

    @pl.when(jnp.logical_and(i >= 0, i < NB - 1))
    @jax.named_scope("p2_b1")
    def _():
        attn = jnp.dot(pqn_scr[...].astype(bf16), m_bf[...], preferred_element_type=f32)
        down_tile(i, 0)
        h_ln(i + 1, attn, 0, TM // 2)
        down_tile(i, 1)
        h_ln(i + 1, attn, TM // 2, TM)
        for j in range(2, NT):
            down_tile(i, j)

    @pl.when(i == NB - 1)
    @jax.named_scope("p2_b2")
    def _():
        for j in range(NT):
            down_tile(i, j)
        for j in range(NT):
            ocopy(i, j).wait()


@jax.jit
def pallas_sequential_preLN__linear_attn_block__glu_gated_reglu__prompt_kernel(
    A_x, A_wqkv, A_wo, B_x, B_W_gate, B_W_up, B_W_down,
):
    bf16 = jnp.bfloat16
    f32 = jnp.float32
    x = A_x.reshape(S, D)
    any_spec = pl.BlockSpec(memory_space=pl.ANY)
    out = pl.pallas_call(
        _kernel,
        grid=(2 * NB + 1,),
        in_specs=[any_spec] * 6,
        out_specs=any_spec,
        out_shape=jax.ShapeDtypeStruct((S, D), A_x.dtype),
        scratch_shapes=[
            pltpu.VMEM((NB, TM, D), bf16),
            pltpu.VMEM((D, D), bf16),
            pltpu.VMEM((D, D), bf16),
            pltpu.VMEM((D, D), bf16),
            pltpu.VMEM((D, D), bf16),
            pltpu.VMEM((D, F), bf16),
            pltpu.VMEM((D, F), bf16),
            pltpu.VMEM((F, D), bf16),
            pltpu.VMEM((D, D), bf16),
            pltpu.VMEM((D, D), bf16),
            pltpu.VMEM((NB, TM, D), bf16),
            pltpu.VMEM((NB, D, TM), f32),
            pltpu.VMEM((D, D), f32),
            pltpu.VMEM((D, 128), f32),
            pltpu.VMEM((D, D), f32),
            pltpu.VMEM((D, D), bf16),
            pltpu.VMEM((D, 128), f32),
            pltpu.VMEM((TM, D), f32),
            pltpu.VMEM((TM, D), f32),
            pltpu.VMEM((TM, D), bf16),
            pltpu.VMEM((TM, F), bf16),
            pltpu.VMEM((TM, D), f32),
            pltpu.VMEM((TM, D), bf16),
            pltpu.VMEM((D, TM), bf16),
            pltpu.SemaphoreType.DMA((NB + 9,)),
            pltpu.SemaphoreType.DMA((NT,)),
        ],
        compiler_params=pltpu.CompilerParams(
            dimension_semantics=("arbitrary",),
            vmem_limit_bytes=100 * 1024 * 1024,
        ),
    )(x, A_wqkv, A_wo, B_W_gate, B_W_up, B_W_down)
    return out.reshape(A_x.shape)
```

```python
import jax
import jax.numpy as jnp
from jax import lax
import jax.experimental.pallas as pl
import jax.experimental.pallas.tpu as pltpu

S = 2048
D = 640
F = 1536
H = 32
DH = D // H
TM = 512
NB = S // TM
HM = TM // 2
NT = D // 128
NP = H // 2
NC = TM // 128
FC = F // NC
KS = 256


def _band(j):
    h0 = (128 * j) // DH
    h1 = (128 * j + 127) // DH
    r0 = (h0 * DH) // 16 * 16
    r1 = -(-((h1 + 1) * DH) // 16) * 16
    return r0, min(r1, D)


BANDS = [_band(j) for j in range(NT)]


def _ln(x):
    mu = jnp.mean(x, axis=-1, keepdims=True)
    xc = x - mu
    var = jnp.mean(xc * xc, axis=-1, keepdims=True)
    return xc * lax.rsqrt(var + 1e-5)


def _recip(d):
    r = pl.reciprocal(d, approx=True)
    return r * (2.0 - d * r)


def _phi(t):
    return jnp.where(t > 0, t + 1.0, jnp.exp(t)) + 1e-6


def _kernel(x_hbm, wqkv_hbm, wo_hbm, wg_hbm, wu_hbm, wd_hbm, o_hbm,
            x_scr, wq, wk, wv, wo, wg, wu, wd, wkT, wqT, xn_scr, pqT_scr, g_acc, z_acc, m_scr, m_bf,
            zb_scr, h_cur, h_nxt, hn_scr, a_scr, pqn_scr, o_scr, pk_scr, sems, osems):
    s = pl.program_id(0)
    f32 = jnp.float32
    bf16 = jnp.bfloat16

    pairs = [(x_hbm.at[pl.ds(0, HM), :], x_scr.at[0, pl.ds(0, HM), :]),
             (wqkv_hbm.at[:, D:D + KS], wk.at[:, 0:KS]),
             (wqkv_hbm.at[:, D + KS:2 * D], wk.at[:, KS:D]),
             (x_hbm.at[pl.ds(HM, HM), :], x_scr.at[0, pl.ds(HM, HM), :]),
             (wqkv_hbm.at[:, 0:D], wq)]
    IQ = len(pairs) - 1
    for b in range(1, NB):
        pairs.append((x_hbm.at[pl.ds(b * TM, TM), :], x_scr.at[b]))
    IREST = len(pairs)
    pairs += [(wqkv_hbm.at[:, 2 * D:3 * D], wv), (wo_hbm, wo), (wg_hbm, wg), (wu_hbm, wu), (wd_hbm, wd)]
    NDMA = len(pairs)

    def copy(n):
        return pltpu.make_async_copy(pairs[n][0], pairs[n][1], sems.at[n])

    def ocopy(blk, j):
        return pltpu.make_async_copy(
            o_scr.at[:, 128 * j:128 * (j + 1)],
            o_hbm.at[pl.ds(pl.multiple_of(blk * TM, TM), TM), 128 * j:128 * (j + 1)],
            osems.at[j])

    NTDIMS = (((1,), (1,)), ((), ()))

    def qproj(blk, r0=0, r1=D):
        qT = lax.dot_general(wqT[r0:r1, :], xn_scr[blk], NTDIMS, preferred_element_type=f32)
        pqT_scr[blk, r0:r1, :] = _phi(qT)

    def lane_fold(t):
        acc = t[:, 0:128]
        for c in range(1, t.shape[1] // 128):
            acc = acc + t[:, 128 * c:128 * (c + 1)]
        return acc

    def norm_piece(blk, c):
        lo = lax.broadcasted_iota(jnp.int32, (NP, 8, 128), 1) < 4
        zb5 = zb_scr[...].reshape(NP, 5, 8, 128)
        p5 = pqT_scr[blk, :, 128 * c:128 * (c + 1)].reshape(NP, 5, 8, 128)
        t5 = p5 * zb5
        ta = t5[:, 0] + t5[:, 1] + jnp.where(lo, t5[:, 2], 0.0)
        tb = jnp.where(lo, 0.0, t5[:, 2]) + t5[:, 3] + t5[:, 4]
        ra = _recip(jnp.sum(ta, axis=1, keepdims=True) + 1e-6)
        rb = _recip(jnp.sum(tb, axis=1, keepdims=True) + 1e-6)
        ra = jnp.broadcast_to(ra, (NP, 8, 128))
        rb = jnp.broadcast_to(rb, (NP, 8, 128))
        rm = jnp.where(lo, ra, rb)
        pn = jnp.stack([p5[:, 0] * ra, p5[:, 1] * ra, p5[:, 2] * rm, p5[:, 3] * rb, p5[:, 4] * rb],
                       axis=1).reshape(D, 128)
        pqn_scr[128 * c:128 * (c + 1), :] = pn.T

    def attn_out():
        return jnp.dot(pqn_scr[...].astype(bf16), m_bf[...], preferred_element_type=f32)

    def h_ln(blk, attn, r0, r1):
        h = x_scr[blk, r0:r1, :].astype(f32) + attn[r0:r1, :]
        h_nxt[r0:r1, :] = h
        hn_scr[r0:r1, :] = _ln(h).astype(bf16)

    def down_tile(blk, j):
        d = jnp.dot(a_scr[...], wd[:, 128 * j:128 * (j + 1)], preferred_element_type=f32)
        o_scr[:, 128 * j:128 * (j + 1)] = (h_cur[:, 128 * j:128 * (j + 1)] + d).astype(bf16)
        ocopy(blk, j).start()

    @pl.when(s == 0)
    def _():
        for n in range(NDMA):
            copy(n).start()

        def kpiece(r0, r1, c0, c1):
            kT = lax.dot_general(wkT[r0:r1, :], xn_scr[0, c0:c1, :], NTDIMS,
                                 preferred_element_type=f32)
            pkT = _phi(kT)
            if c0 == 0:
                z_acc[r0:r1, :] = lane_fold(pkT)
            else:
                z_acc[r0:r1, :] += lane_fold(pkT)
            pk_scr[r0:r1, c0:c1] = pkT.astype(bf16)

        copy(0).wait()
        xn_scr[0, 0:HM, :] = _ln(x_scr[0, 0:HM, :].astype(f32)).astype(bf16)
        copy(1).wait()
        wkT[0:KS, :] = wk[:, 0:KS].T
        kpiece(0, KS, 0, HM)
        copy(2).wait()
        copy(3).wait()
        wkT[KS:D, :] = wk[:, KS:D].T
        xn_scr[0, HM:TM, :] = _ln(x_scr[0, HM:TM, :].astype(f32)).astype(bf16)
        kpiece(KS, D, 0, HM)
        kpiece(0, D, HM, TM)
        copy(IQ).wait()
        wqT[...] = wq[...].T
        g_acc[...] = jnp.dot(pk_scr[...], xn_scr[0], preferred_element_type=f32)

    @pl.when(jnp.logical_and(s > 0, s < NB))
    def _():
        pltpu.make_async_copy(x_hbm.at[pl.ds(pl.multiple_of(s * TM, TM), TM), :], x_scr.at[s],
                              sems.at[s + IQ]).wait()
        qproj(s - 1)
        xn = _ln(x_scr[s].astype(f32)).astype(bf16)
        xn_scr[s] = xn
        kT = lax.dot_general(wkT[...], xn, NTDIMS, preferred_element_type=f32)
        pkT = _phi(kT)
        z_acc[...] += lane_fold(pkT)
        g_acc[...] += jnp.dot(pkT.astype(bf16), xn, preferred_element_type=f32)

    @pl.when(s == NB)
    def _():
        for n in range(IREST, NDMA):
            copy(n).wait()
        zb_scr[...] = jnp.broadcast_to(jnp.sum(z_acc[...], axis=1, keepdims=True), (D, 128))
        kvs = []
        for j, (r0, r1) in enumerate(BANDS):
            n = r1 - r0
            kvj = jnp.dot(g_acc[r0:r1, :].astype(bf16), wv[:, 128 * j:128 * (j + 1)],
                          preferred_element_type=f32)
            rh = (lax.broadcasted_iota(jnp.int32, (n, 128), 0) + r0) // DH
            ch = (lax.broadcasted_iota(jnp.int32, (n, 128), 1) + 128 * j) // DH
            kvs.append(jnp.where(rh == ch, kvj, 0.0).astype(bf16))
        for c in range(NC):
            norm_piece(0, c)
        qproj(NB - 1, 0, 256)
        m_scr[...] = jnp.zeros(m_scr.shape, f32)
        for j, (r0, r1) in enumerate(BANDS):
            m_scr[r0:r1, :] += jnp.dot(kvs[j], wo[128 * j:128 * (j + 1), :], preferred_element_type=f32)
        qproj(NB - 1, 256, 384)
        m_bf[...] = m_scr[...].astype(bf16)
        attn = attn_out()
        qproj(NB - 1, 384, D)
        h_ln(0, attn, 0, TM)

    i = s - (NB + 1)

    @pl.when(i >= 0)
    def _():
        h_cur[...] = h_nxt[...]
        hn = hn_scr[...]
        nxt = jnp.minimum(i + 1, NB - 1)
        for c in range(NC):
            g = jnp.dot(hn, wg[:, FC * c:FC * (c + 1)], preferred_element_type=f32)
            u = jnp.dot(hn, wu[:, FC * c:FC * (c + 1)], preferred_element_type=f32)
            norm_piece(nxt, c)
            a_scr[:, FC * c:FC * (c + 1)] = (jnp.maximum(g, 0.0) * u).astype(bf16)

    @pl.when(i >= 1)
    def _():
        for j in range(NT):
            ocopy(i - 1, j).wait()

    @pl.when(jnp.logical_and(i >= 0, i < NB - 1))
    def _():
        attn = attn_out()
        for j in range(NT):
            down_tile(i, j)
            if j < NC:
                h_ln(i + 1, attn, 128 * j, 128 * (j + 1))

    @pl.when(i == NB - 1)
    def _():
        for j in range(NT):
            down_tile(i, j)
        for j in range(NT):
            ocopy(i, j).wait()


@jax.jit
def pallas_sequential_preLN__linear_attn_block__glu_gated_reglu__prompt_kernel(
    A_x: jax.Array,
    A_wqkv: jax.Array,
    A_wo: jax.Array,
    B_x: jax.Array,
    B_W_gate: jax.Array,
    B_W_up: jax.Array,
    B_W_down: jax.Array,
):
    del B_x
    bf16 = jnp.bfloat16
    f32 = jnp.float32
    x = A_x.reshape(S, D)
    any_spec = pl.BlockSpec(memory_space=pl.ANY)
    out = pl.pallas_call(
        _kernel,
        grid=(2 * NB + 1,),
        in_specs=[any_spec] * 6,
        out_specs=any_spec,
        out_shape=jax.ShapeDtypeStruct((S, D), A_x.dtype),
        scratch_shapes=[
            pltpu.VMEM((NB, TM, D), bf16),
            pltpu.VMEM((D, D), bf16),
            pltpu.VMEM((D, D), bf16),
            pltpu.VMEM((D, D), bf16),
            pltpu.VMEM((D, D), bf16),
            pltpu.VMEM((D, F), bf16),
            pltpu.VMEM((D, F), bf16),
            pltpu.VMEM((F, D), bf16),
            pltpu.VMEM((D, D), bf16),
            pltpu.VMEM((D, D), bf16),
            pltpu.VMEM((NB, TM, D), bf16),
            pltpu.VMEM((NB, D, TM), f32),
            pltpu.VMEM((D, D), f32),
            pltpu.VMEM((D, 128), f32),
            pltpu.VMEM((D, D), f32),
            pltpu.VMEM((D, D), bf16),
            pltpu.VMEM((D, 128), f32),
            pltpu.VMEM((TM, D), f32),
            pltpu.VMEM((TM, D), f32),
            pltpu.VMEM((TM, D), bf16),
            pltpu.VMEM((TM, F), bf16),
            pltpu.VMEM((TM, D), f32),
            pltpu.VMEM((TM, D), bf16),
            pltpu.VMEM((D, TM), bf16),
            pltpu.SemaphoreType.DMA((NB + 9,)),
            pltpu.SemaphoreType.DMA((NT,)),
        ],
        compiler_params=pltpu.CompilerParams(
            dimension_semantics=("arbitrary",),
            vmem_limit_bytes=100 * 1024 * 1024,
        ),
    )(x, A_wqkv, A_wo, B_W_gate, B_W_up, B_W_down)
    return out.reshape(A_x.shape)
```

```python
import jax
import jax.numpy as jnp
from jax import lax
import jax.experimental.pallas as pl
import jax.experimental.pallas.tpu as pltpu

S = 2048
D = 640
F = 1536
H = 32
DH = D // H
TM = 512
NB = S // TM
HM = TM // 2
NT = D // 128
NP = H // 2
NC = TM // 128
FC = F // NC
KS = 256


def _band(j):
    h0 = (128 * j) // DH
    h1 = (128 * j + 127) // DH
    r0 = (h0 * DH) // 16 * 16
    r1 = -(-((h1 + 1) * DH) // 16) * 16
    return r0, min(r1, D)


BANDS = [_band(j) for j in range(NT)]


def _ln(x):
    mu = jnp.mean(x, axis=-1, keepdims=True)
    xc = x - mu
    var = jnp.mean(xc * xc, axis=-1, keepdims=True)
    return xc * lax.rsqrt(var + 1e-5)


def _recip(d):
    r = pl.reciprocal(d, approx=True)
    return r * (2.0 - d * r)


def _phi(t):
    return jnp.where(t > 0, t + 1.0, jnp.exp(t)) + 1e-6


def _kernel(x_hbm, wqkv_hbm, wo_hbm, wg_hbm, wu_hbm, wd_hbm, o_hbm,
            x_scr, wq, wk, wv, wo, wg, wu, wd, wkT, wqT, xn_scr, pqT_scr, g_acc, z_acc, m_scr, m_bf,
            zb_scr, h_cur, h_nxt, hn_scr, a_scr, pqn_scr, o_scr, pk_scr, sems, osems):
    s = pl.program_id(0)
    f32 = jnp.float32
    bf16 = jnp.bfloat16

    pairs = [(x_hbm.at[pl.ds(0, HM), :], x_scr.at[0, pl.ds(0, HM), :]),
             (wqkv_hbm.at[:, D:D + KS], wk.at[:, 0:KS]),
             (wqkv_hbm.at[:, D + KS:2 * D], wk.at[:, KS:D]),
             (x_hbm.at[pl.ds(HM, HM), :], x_scr.at[0, pl.ds(HM, HM), :]),
             (wqkv_hbm.at[:, 0:D], wq)]
    IQ = len(pairs) - 1
    for b in range(1, NB):
        pairs.append((x_hbm.at[pl.ds(b * TM, TM), :], x_scr.at[b]))
    IREST = len(pairs)
    pairs += [(wqkv_hbm.at[:, 2 * D:3 * D], wv), (wo_hbm, wo), (wg_hbm, wg), (wu_hbm, wu), (wd_hbm, wd)]
    NDMA = len(pairs)

    def copy(n):
        return pltpu.make_async_copy(pairs[n][0], pairs[n][1], sems.at[n])

    def ocopy(blk, j):
        slot = blk % 2
        return pltpu.make_async_copy(
            o_scr.at[slot, :, 128 * j:128 * (j + 1)],
            o_hbm.at[pl.ds(pl.multiple_of(blk * TM, TM), TM), 128 * j:128 * (j + 1)],
            osems.at[slot * NT + j])

    NTDIMS = (((1,), (1,)), ((), ()))

    def qproj(blk, r0=0, r1=D):
        qT = lax.dot_general(wqT[r0:r1, :], xn_scr[blk], NTDIMS, preferred_element_type=f32)
        pqT_scr[blk, r0:r1, :] = _phi(qT)

    def lane_fold(t):
        acc = t[:, 0:128]
        for c in range(1, t.shape[1] // 128):
            acc = acc + t[:, 128 * c:128 * (c + 1)]
        return acc

    def norm_piece(blk, c):
        lo = lax.broadcasted_iota(jnp.int32, (NP, 8, 128), 1) < 4
        zb5 = zb_scr[...].reshape(NP, 5, 8, 128)
        p5 = pqT_scr[blk, :, 128 * c:128 * (c + 1)].reshape(NP, 5, 8, 128)
        t5 = p5 * zb5
        ta = t5[:, 0] + t5[:, 1] + jnp.where(lo, t5[:, 2], 0.0)
        tb = jnp.where(lo, 0.0, t5[:, 2]) + t5[:, 3] + t5[:, 4]
        ra = _recip(jnp.sum(ta, axis=1, keepdims=True) + 1e-6)
        rb = _recip(jnp.sum(tb, axis=1, keepdims=True) + 1e-6)
        ra = jnp.broadcast_to(ra, (NP, 8, 128))
        rb = jnp.broadcast_to(rb, (NP, 8, 128))
        rm = jnp.where(lo, ra, rb)
        pn = jnp.stack([p5[:, 0] * ra, p5[:, 1] * ra, p5[:, 2] * rm, p5[:, 3] * rb, p5[:, 4] * rb],
                       axis=1).reshape(D, 128)
        pqn_scr[128 * c:128 * (c + 1), :] = pn.T

    def attn_out():
        return jnp.dot(pqn_scr[...].astype(bf16), m_bf[...], preferred_element_type=f32)

    def h_ln(blk, attn, r0, r1):
        h = x_scr[blk, r0:r1, :].astype(f32) + attn[r0:r1, :]
        h_nxt[r0:r1, :] = h
        hn_scr[r0:r1, :] = _ln(h).astype(bf16)

    def down_tile(blk, j):
        d = jnp.dot(a_scr[...], wd[:, 128 * j:128 * (j + 1)], preferred_element_type=f32)
        o_scr[blk % 2, :, 128 * j:128 * (j + 1)] = (h_cur[:, 128 * j:128 * (j + 1)] + d).astype(bf16)
        ocopy(blk, j).start()

    @pl.when(s == 0)
    def _():
        for n in range(NDMA):
            copy(n).start()

        def kpiece(r0, r1, c0, c1):
            kT = lax.dot_general(wkT[r0:r1, :], xn_scr[0, c0:c1, :], NTDIMS,
                                 preferred_element_type=f32)
            pkT = _phi(kT)
            if c0 == 0:
                z_acc[r0:r1, :] = lane_fold(pkT)
            else:
                z_acc[r0:r1, :] += lane_fold(pkT)
            pk_scr[r0:r1, c0:c1] = pkT.astype(bf16)

        copy(0).wait()
        xn_scr[0, 0:HM, :] = _ln(x_scr[0, 0:HM, :].astype(f32)).astype(bf16)
        copy(1).wait()
        wkT[0:KS, :] = wk[:, 0:KS].T
        kpiece(0, KS, 0, HM)
        copy(2).wait()
        copy(3).wait()
        wkT[KS:D, :] = wk[:, KS:D].T
        xn_scr[0, HM:TM, :] = _ln(x_scr[0, HM:TM, :].astype(f32)).astype(bf16)
        kpiece(KS, D, 0, HM)
        kpiece(0, D, HM, TM)
        copy(IQ).wait()
        wqT[...] = wq[...].T
        g_acc[...] = jnp.dot(pk_scr[...], xn_scr[0], preferred_element_type=f32)

    @pl.when(jnp.logical_and(s > 0, s < NB))
    def _():
        pltpu.make_async_copy(x_hbm.at[pl.ds(pl.multiple_of(s * TM, TM), TM), :], x_scr.at[s],
                              sems.at[s + IQ]).wait()
        qproj(s - 1)
        xn = _ln(x_scr[s].astype(f32)).astype(bf16)
        xn_scr[s] = xn
        kT = lax.dot_general(wkT[...], xn, NTDIMS, preferred_element_type=f32)
        pkT = _phi(kT)
        z_acc[...] += lane_fold(pkT)
        g_acc[...] += jnp.dot(pkT.astype(bf16), xn, preferred_element_type=f32)

    @pl.when(s == NB)
    def _():
        for n in range(IREST, NDMA):
            copy(n).wait()
        zb_scr[...] = jnp.broadcast_to(jnp.sum(z_acc[...], axis=1, keepdims=True), (D, 128))
        kvs = []
        for j, (r0, r1) in enumerate(BANDS):
            n = r1 - r0
            kvj = jnp.dot(g_acc[r0:r1, :].astype(bf16), wv[:, 128 * j:128 * (j + 1)],
                          preferred_element_type=f32)
            rh = (lax.broadcasted_iota(jnp.int32, (n, 128), 0) + r0) // DH
            ch = (lax.broadcasted_iota(jnp.int32, (n, 128), 1) + 128 * j) // DH
            kvs.append(jnp.where(rh == ch, kvj, 0.0).astype(bf16))
        for c in range(NC):
            norm_piece(0, c)
        qproj(NB - 1, 0, 256)
        m_scr[...] = jnp.zeros(m_scr.shape, f32)
        for j, (r0, r1) in enumerate(BANDS):
            m_scr[r0:r1, :] += jnp.dot(kvs[j], wo[128 * j:128 * (j + 1), :], preferred_element_type=f32)
        qproj(NB - 1, 256, 384)
        m_bf[...] = m_scr[...].astype(bf16)
        attn = attn_out()
        qproj(NB - 1, 384, D)
        h_ln(0, attn, 0, TM)

    hf = s - (NB + 1)

    @pl.when(jnp.logical_and(hf >= 0, hf < 2))
    def _():
        rows = pl.ds(pl.multiple_of(hf * HM, HM), HM)
        h_cur[rows, :] = h_nxt[rows, :]
        hn = hn_scr[rows, :]
        for c in range(NC):
            g = jnp.dot(hn, wg[:, FC * c:FC * (c + 1)], preferred_element_type=f32)
            u = jnp.dot(hn, wu[:, FC * c:FC * (c + 1)], preferred_element_type=f32)
            a_scr[rows, FC * c:FC * (c + 1)] = (jnp.maximum(g, 0.0) * u).astype(bf16)
        for c in range(NC):
            norm_piece(1, c)

    i = s - (NB + 3)

    @pl.when(i >= 2)
    def _():
        for j in range(NT):
            ocopy(i - 2, j).wait()

    @pl.when(jnp.logical_and(i >= 0, i < NB - 1))
    def _():
        attn = attn_out()
        for j in range(NT):
            down_tile(i, j)
            if j < NC:
                h_ln(i + 1, attn, 128 * j, 128 * (j + 1))
        h_cur[...] = h_nxt[...]
        hn = hn_scr[...]
        nxt = jnp.minimum(i + 2, NB - 1)
        for c in range(NC):
            g = jnp.dot(hn, wg[:, FC * c:FC * (c + 1)], preferred_element_type=f32)
            u = jnp.dot(hn, wu[:, FC * c:FC * (c + 1)], preferred_element_type=f32)
            norm_piece(nxt, c)
            a_scr[:, FC * c:FC * (c + 1)] = (jnp.maximum(g, 0.0) * u).astype(bf16)

    @pl.when(i == NB - 1)
    def _():
        for j in range(NT):
            down_tile(i, j)
        for j in range(NT):
            ocopy(i - 1, j).wait()
        for j in range(NT):
            ocopy(i, j).wait()


@jax.jit
def pallas_sequential_preLN__linear_attn_block__glu_gated_reglu__prompt_kernel(
    A_x: jax.Array,
    A_wqkv: jax.Array,
    A_wo: jax.Array,
    B_x: jax.Array,
    B_W_gate: jax.Array,
    B_W_up: jax.Array,
    B_W_down: jax.Array,
):
    del B_x
    bf16 = jnp.bfloat16
    f32 = jnp.float32
    x = A_x.reshape(S, D)
    any_spec = pl.BlockSpec(memory_space=pl.ANY)
    out = pl.pallas_call(
        _kernel,
        grid=(2 * NB + 3,),
        in_specs=[any_spec] * 6,
        out_specs=any_spec,
        out_shape=jax.ShapeDtypeStruct((S, D), A_x.dtype),
        scratch_shapes=[
            pltpu.VMEM((NB, TM, D), bf16),
            pltpu.VMEM((D, D), bf16),
            pltpu.VMEM((D, D), bf16),
            pltpu.VMEM((D, D), bf16),
            pltpu.VMEM((D, D), bf16),
            pltpu.VMEM((D, F), bf16),
            pltpu.VMEM((D, F), bf16),
            pltpu.VMEM((F, D), bf16),
            pltpu.VMEM((D, D), bf16),
            pltpu.VMEM((D, D), bf16),
            pltpu.VMEM((NB, TM, D), bf16),
            pltpu.VMEM((NB, D, TM), f32),
            pltpu.VMEM((D, D), f32),
            pltpu.VMEM((D, 128), f32),
            pltpu.VMEM((D, D), f32),
            pltpu.VMEM((D, D), bf16),
            pltpu.VMEM((D, 128), f32),
            pltpu.VMEM((TM, D), f32),
            pltpu.VMEM((TM, D), f32),
            pltpu.VMEM((TM, D), bf16),
            pltpu.VMEM((TM, F), bf16),
            pltpu.VMEM((TM, D), f32),
            pltpu.VMEM((2, TM, D), bf16),
            pltpu.VMEM((D, TM), bf16),
            pltpu.SemaphoreType.DMA((NB + 9,)),
            pltpu.SemaphoreType.DMA((2 * NT,)),
        ],
        compiler_params=pltpu.CompilerParams(
            dimension_semantics=("arbitrary",),
            vmem_limit_bytes=100 * 1024 * 1024,
        ),
    )(x, A_wqkv, A_wo, B_W_gate, B_W_up, B_W_down)
    return out.reshape(A_x.shape)
```
